```python
import jax
import jax.numpy as jnp

def _softmax(x, axis=-1):
    return jax.nn.softmax(x, axis=axis)
def _gelu(x):
    return jax.nn.gelu(x, approximate=True)
def _silu(x):
    return jax.nn.silu(x)
def _sigmoid(x):
    return jax.nn.sigmoid(x)
def _layernorm(x, axis=-1, eps=1e-5):
    m = jnp.mean(x, axis=axis, keepdims=True)
    v = jnp.var(x, axis=axis, keepdims=True)
    return (x - m) / jnp.sqrt(v + eps)
def _scatter_add(tgt, idx, src, axis=0):
    return tgt.at[idx].add(src)
def _segment_sum(src, seg, n):
    return jax.ops.segment_sum(src, seg, n)
class _Rng:
    def __init__(self, key):
        self._k = key
    def _next(self):
        self._k, sub = jax.random.split(self._k)
        return sub
    def normal(self, shape):
        return jax.random.normal(self._next(), shape, dtype=jnp.bfloat16)
    def randint(self, lo, hi, shape):
        return jax.random.randint(self._next(), shape, lo, hi, dtype=jnp.int32)
    def uniform(self, shape, lo=0.0, hi=1.0):
        return jax.random.uniform(self._next(), shape, jnp.bfloat16, lo, hi)
    def permutation(self, n):
        return jax.random.permutation(self._next(), n)


kernel_name = 'standalone__modern_conv_block_replknet__vision'

def setup_inputs():
    _rng = _Rng(jax.random.key(int.from_bytes(__import__("os").urandom(4), "little")))
    _w = (lambda a: (lambda t: t.astype(jnp.bfloat16) if jnp.issubdtype(t.dtype, jnp.floating) else t)(jnp.asarray(a)))
    H = W = 512
    C = 96
    K = 3
    return {
        "x": _w((lambda *s: _rng.normal(s) * 0.05)(1, H, W, C)),
        "dw_large": _w((lambda *s: _rng.normal(s) * 0.05)(K, K, C) * (1.0 / K)),
        "dw_small": _w((lambda *s: _rng.normal(s) * 0.05)(5, 5, C) * 0.2),
        "w1": _w((lambda *s: _rng.normal(s) * 0.05)(C, 4 * C) * (C ** -0.5)),
        "w2": _w((lambda *s: _rng.normal(s) * 0.05)(4 * C, C) * ((4 * C) ** -0.5)),
    }

def reference(x, dw_large, dw_small, w1, w2):
    B, H, W, C = x.shape
    Kl = dw_large.shape[0]
    pl = (Kl - 1) // 2
    xpl = jnp.pad(x, ((0,0),(pl,pl),(pl,pl),(0,0)))
    out = jnp.zeros_like(x)
    for i in range(Kl):
        for j in range(Kl):
            out = out + xpl[:, i:i+H, j:j+W, :] * dw_large[i, j][None, None, None, :]
    Ks = dw_small.shape[0]
    ps = (Ks - 1) // 2
    xps = jnp.pad(x, ((0,0),(ps,ps),(ps,ps),(0,0)))
    for i in range(Ks):
        for j in range(Ks):
            out = out + xps[:, i:i+H, j:j+W, :] * dw_small[i, j][None, None, None, :]
    h = _layernorm(out, axis=-1)
    h = _gelu(jnp.einsum('bhwc,ce->bhwe', h, w1))
    h = jnp.einsum('bhwe,ec->bhwc', h, w2)
    return x + h
```

```python
import jax
import jax.numpy as jnp
import numpy as np
import jax.experimental.pallas as pl
import jax.experimental.pallas.tpu as pltpu

TH = 32
_C2 = float(np.sqrt(2.0 / np.pi) * 0.044715)
_A = float(_C2 ** (1.0 / 3.0))
_B = float(np.sqrt(2.0 / np.pi) / _A)


def _kernel(xm_ref, xt_ref, xb_ref, dl_ref, ds_ref, w1_ref, w2t_ref, o_ref,
            kw_s, w1t_s, xs_s):
    i = pl.program_id(0)
    n = pl.num_programs(0)
    C, W = xm_ref.shape[1], xm_ref.shape[2]

    @pl.when(i == 0)
    def _():
        ds = ds_ref[...].astype(jnp.float32)
        dl = dl_ref[...].astype(jnp.float32)
        for a in range(5):
            for b in range(5):
                k = ds[a, b:b + 1, :]
                if 1 <= a <= 3 and 1 <= b <= 3:
                    k = k + dl[a - 1, b - 1:b, :]
                kb = jnp.broadcast_to(k, (128, C))
                kw_s[a * 5 + b] = kb.T
        w1t_s[...] = w1_ref[...].astype(jnp.float32).T.astype(jnp.bfloat16)

    xs_s[0:2] = jnp.where(i > 0, xt_ref[...].astype(jnp.float32), 0.0)
    xs_s[2:TH + 2] = xm_ref[...].astype(jnp.float32)
    xs_s[TH + 2:TH + 4] = jnp.where(i < n - 1, xb_ref[...].astype(jnp.float32), 0.0)

    lane = jax.lax.broadcasted_iota(jnp.int32, (8, W), 1)

    def body(r, carry):
        outs = []
        for g in range(C // 8):
            rows = [xs_s[r + a, g * 8:(g + 1) * 8, :] for a in range(5)]
            acc = None
            for b in range(5):
                t = None
                for a in range(5):
                    k = kw_s[a * 5 + b, g * 8:(g + 1) * 8, :]
                    k = jnp.concatenate([k] * (W // 128), axis=1)
                    p = rows[a] * k
                    t = p if t is None else t + p
                s = b - 2
                if s != 0:
                    t = pltpu.roll(t, (-s) % W, 1)
                    if s > 0:
                        t = jnp.where(lane < W - s, t, 0.0)
                    else:
                        t = jnp.where(lane >= -s, t, 0.0)
                acc = t if acc is None else acc + t
            outs.append(acc)
        c = jnp.concatenate(outs, axis=0)
        m = jnp.sum(c, axis=0, keepdims=True) * (1.0 / C)
        d = c - m
        v = jnp.sum(d * d, axis=0, keepdims=True) * (1.0 / C)
        h = (d * (jax.lax.rsqrt(v + 1e-5) * _A)).astype(jnp.bfloat16)
        y = jnp.dot(w1t_s[...], h, preferred_element_type=jnp.float32)
        t = jnp.tanh(y * (y * y + _B))
        gl = (y + y * t).astype(jnp.bfloat16)
        o = jnp.dot(w2t_ref[...], gl, preferred_element_type=jnp.float32)
        o_ref[r] = (xs_s[r + 2] + o * (0.5 / _A)).astype(o_ref.dtype)
        return carry

    jax.lax.fori_loop(0, TH, body, 0)


@jax.jit
def pallas_standalone__modern_conv_block_replknet__vision_kernel(x, dw_large, dw_small, w1, w2):
    B, H, W, C = x.shape
    xt = jnp.transpose(x, (0, 1, 3, 2)).reshape(B * H, C, W)
    E = w1.shape[1]
    n = H // TH
    out = pl.pallas_call(
        _kernel,
        grid=(n,),
        in_specs=[
            pl.BlockSpec((TH, C, W), lambda i: (i, 0, 0)),
            pl.BlockSpec((2, C, W), lambda i: (jnp.maximum(i * (TH // 2) - 1, 0), 0, 0)),
            pl.BlockSpec((2, C, W), lambda i: (jnp.minimum((i + 1) * (TH // 2), H // 2 - 1), 0, 0)),
            pl.BlockSpec(dw_large.shape, lambda i: (0, 0, 0)),
            pl.BlockSpec(dw_small.shape, lambda i: (0, 0, 0)),
            pl.BlockSpec((C, E), lambda i: (0, 0)),
            pl.BlockSpec((C, E), lambda i: (0, 0)),
        ],
        out_specs=pl.BlockSpec((TH, C, W), lambda i: (i, 0, 0)),
        out_shape=jax.ShapeDtypeStruct((B * H, C, W), x.dtype),
        scratch_shapes=[
            pltpu.VMEM((25, C, 128), jnp.float32),
            pltpu.VMEM((E, C), jnp.bfloat16),
            pltpu.VMEM((TH + 4, C, W), jnp.float32),
        ],
        compiler_params=pltpu.CompilerParams(
            dimension_semantics=("arbitrary",), vmem_limit_bytes=64 * 1024 * 1024),
    )(xt, xt, xt, dw_large, dw_small, w1, w2.T)
    return jnp.transpose(out.reshape(B, H, C, W), (0, 1, 3, 2))
```

```python
import jax
import jax.numpy as jnp
import numpy as np
import jax.experimental.pallas as pl
import jax.experimental.pallas.tpu as pltpu

TH = 64
_C2 = float(np.sqrt(2.0 / np.pi) * 0.044715)
_A = float(_C2 ** (1.0 / 3.0))
_B = float(np.sqrt(2.0 / np.pi) / _A)


def _kernel(xm_ref, xt_ref, xb_ref, dl_ref, ds_ref, w1_ref, w2t_ref, o_ref,
            kw_s, w1t_s, xs_s, h_s, g_s):
    i = pl.program_id(0)
    n = pl.num_programs(0)
    C, W = xm_ref.shape[1], xm_ref.shape[2]

    @pl.when(i == 0)
    def _():
        ds = ds_ref[...].astype(jnp.float32)
        dl = dl_ref[...].astype(jnp.float32)
        for a in range(5):
            for b in range(5):
                k = ds[a, b:b + 1, :]
                if 1 <= a <= 3 and 1 <= b <= 3:
                    k = k + dl[a - 1, b - 1:b, :]
                kb = jnp.broadcast_to(k, (128, C))
                kw_s[a * 5 + b] = kb.T
        w1t_s[...] = w1_ref[...].astype(jnp.float32).T.astype(jnp.bfloat16)

    xs_s[0:2] = jnp.where(i > 0, xt_ref[...].astype(jnp.float32), 0.0)
    xs_s[2:TH + 2] = xm_ref[...].astype(jnp.float32)
    xs_s[TH + 2:TH + 4] = jnp.where(i < n - 1, xb_ref[...].astype(jnp.float32), 0.0)

    lane = jax.lax.broadcasted_iota(jnp.int32, (8, W), 1)

    def conv(r):
        outs = []
        for g in range(C // 8):
            rows = [xs_s[r + a, g * 8:(g + 1) * 8, :] for a in range(5)]
            acc = None
            for b in range(5):
                t = None
                for a in range(5):
                    k = kw_s[a * 5 + b, g * 8:(g + 1) * 8, :]
                    k = jnp.concatenate([k] * (W // 128), axis=1)
                    p = rows[a] * k
                    t = p if t is None else t + p
                s = b - 2
                if s != 0:
                    t = pltpu.roll(t, (-s) % W, 1)
                    if s > 0:
                        t = jnp.where(lane < W - s, t, 0.0)
                    else:
                        t = jnp.where(lane >= -s, t, 0.0)
                acc = t if acc is None else acc + t
            outs.append(acc)
        c = jnp.concatenate(outs, axis=0)
        m = jnp.sum(c, axis=0, keepdims=True) * (1.0 / C)
        d = c - m
        v = jnp.sum(d * d, axis=0, keepdims=True) * (1.0 / C)
        h = (d * (jax.lax.rsqrt(v + 1e-5) * _A)).astype(jnp.bfloat16)
        return h

    def up(h):
        y = jnp.dot(w1t_s[...], h, preferred_element_type=jnp.float32)
        t = jnp.tanh(y * (y * y + _B))
        return (y + y * t).astype(jnp.bfloat16)

    g_s[0] = up(conv(0))
    h_s[1] = conv(1)

    def body(r, carry):
        p = r % 2
        gl = g_s[p]
        h = h_s[1 - p]
        o = jnp.dot(w2t_ref[...], gl, preferred_element_type=jnp.float32)
        o_ref[r] = (xs_s[r + 2] + o * (0.5 / _A)).astype(o_ref.dtype)
        g_s[1 - p] = up(h)
        h_s[p] = conv(jnp.minimum(r + 2, TH - 1))
        return carry

    jax.lax.fori_loop(0, TH, body, 0)


@jax.jit
def pallas_standalone__modern_conv_block_replknet__vision_kernel(x, dw_large, dw_small, w1, w2):
    B, H, W, C = x.shape
    xt = jnp.transpose(x, (0, 1, 3, 2)).reshape(B * H, C, W)
    E = w1.shape[1]
    n = H // TH
    out = pl.pallas_call(
        _kernel,
        grid=(n,),
        in_specs=[
            pl.BlockSpec((TH, C, W), lambda i: (i, 0, 0)),
            pl.BlockSpec((2, C, W), lambda i: (jnp.maximum(i * (TH // 2) - 1, 0), 0, 0)),
            pl.BlockSpec((2, C, W), lambda i: (jnp.minimum((i + 1) * (TH // 2), H // 2 - 1), 0, 0)),
            pl.BlockSpec(dw_large.shape, lambda i: (0, 0, 0)),
            pl.BlockSpec(dw_small.shape, lambda i: (0, 0, 0)),
            pl.BlockSpec((C, E), lambda i: (0, 0)),
            pl.BlockSpec((C, E), lambda i: (0, 0)),
        ],
        out_specs=pl.BlockSpec((TH, C, W), lambda i: (i, 0, 0)),
        out_shape=jax.ShapeDtypeStruct((B * H, C, W), x.dtype),
        scratch_shapes=[
            pltpu.VMEM((25, C, 128), jnp.float32),
            pltpu.VMEM((E, C), jnp.bfloat16),
            pltpu.VMEM((TH + 4, C, W), jnp.float32),
            pltpu.VMEM((2, C, W), jnp.bfloat16),
            pltpu.VMEM((2, E, W), jnp.bfloat16),
        ],
        compiler_params=pltpu.CompilerParams(
            dimension_semantics=("arbitrary",), vmem_limit_bytes=100 * 1024 * 1024),
    )(xt, xt, xt, dw_large, dw_small, w1, w2.T)
    return jnp.transpose(out.reshape(B, H, C, W), (0, 1, 3, 2))
```
